```python
import os as _os
_os.environ.setdefault("JAX_PLATFORMS", "cpu")
import jax
import jax.numpy as jnp

def _softmax(x, axis=-1):
    return jax.nn.softmax(x, axis=axis)
def _gelu(x):
    return jax.nn.gelu(x, approximate=True)
def _silu(x):
    return jax.nn.silu(x)
def _sigmoid(x):
    return jax.nn.sigmoid(x)
def _layernorm(x, axis=-1, eps=1e-5):
    m = jnp.mean(x, axis=axis, keepdims=True)
    v = jnp.var(x, axis=axis, keepdims=True)
    return (x - m) / jnp.sqrt(v + eps)
def _scatter_add(tgt, idx, src, axis=0):
    return tgt.at[idx].add(src)
def _segment_sum(src, seg, n):
    return jax.ops.segment_sum(src, seg, n)
class _Rng:
    def __init__(self, key):
        self._k = key
    def _next(self):
        self._k, sub = jax.random.split(self._k)
        return sub
    def normal(self, shape):
        return jax.random.normal(self._next(), shape, dtype=jnp.bfloat16)
    def randint(self, lo, hi, shape):
        return jax.random.randint(self._next(), shape, lo, hi, dtype=jnp.int32)
    def uniform(self, shape, lo=0.0, hi=1.0):
        return jax.random.uniform(self._next(), shape, jnp.bfloat16, lo, hi)
    def permutation(self, n):
        return jax.random.permutation(self._next(), n)


kernel_name = 'concat_heads__mha_block_cached__mha_block_cached__near_ridge'

def setup_inputs():
    _rng = _Rng(jax.random.key(int.from_bytes(__import__("os").urandom(4), "little")))
    _w = (lambda a: (lambda t: t.astype(jnp.bfloat16) if jnp.issubdtype(t.dtype, jnp.floating) else t)(jnp.asarray(a)))
    def _A_setup():
        B, Sq, D = 16, 32, 1024
        H, Sk, Dh = 32, 32, 128
        return {
            "x": _w((lambda *s: _rng.normal(s) * 0.8)(B, Sq, D)),
            "k_cache": _w((lambda *s: _rng.normal(s) * 0.8)(B, H, Sk, Dh)),
            "v_cache": _w((lambda *s: _rng.normal(s) * 0.05)(B, H, Sk, Dh)),
            "wq": _w((lambda *s: _rng.normal(s) * 0.8)(D, H * Dh) * (D ** -0.5)),
            "wo": _w((lambda *s: _rng.normal(s) * 0.05)(H * Dh, D) * ((H * Dh) ** -0.5)),
        }
    _A_in = _A_setup()

    def _B_setup():
        B, Sq, D = 16, 32, 1024
        H, Sk, Dh = 32, 32, 128
        return {
            "x": _w((lambda *s: _rng.normal(s) * 0.8)(B, Sq, D)),
            "k_cache": _w((lambda *s: _rng.normal(s) * 0.8)(B, H, Sk, Dh)),
            "v_cache": _w((lambda *s: _rng.normal(s) * 0.05)(B, H, Sk, Dh)),
            "wq": _w((lambda *s: _rng.normal(s) * 0.8)(D, H * Dh) * (D ** -0.5)),
            "wo": _w((lambda *s: _rng.normal(s) * 0.05)(H * Dh, D) * ((H * Dh) ** -0.5)),
        }
    _B_in = _B_setup()

    return {
        "A_x": _A_in["x"],
        "A_k_cache": _A_in["k_cache"],
        "A_v_cache": _A_in["v_cache"],
        "A_wq": _A_in["wq"],
        "A_wo": _A_in["wo"],
        "B_x": _B_in["x"],
        "B_k_cache": _B_in["k_cache"],
        "B_v_cache": _B_in["v_cache"],
        "B_wq": _B_in["wq"],
        "B_wo": _B_in["wo"],
    }

def reference(A_x, A_k_cache, A_v_cache, A_wq, A_wo, B_x, B_k_cache, B_v_cache, B_wq, B_wo):
    def _A_ref(x, k_cache, v_cache, wq, wo):
        B, Sq, D = x.shape
        H, Dh = 32, 128
        q = (lambda x, *d: x.transpose(*d))((x @ wq).reshape(B, Sq, H, Dh), 0, 2, 1, 3)
        scores = jnp.einsum("bhqd,bhkd->bhqk", q, k_cache) * (Dh ** -0.5)
        p = _softmax(scores, axis=-1)
        o = jnp.einsum("bhqk,bhkd->bhqd", p, v_cache)
        return (lambda x, *d: x.transpose(*d))(o, 0, 2, 1, 3).reshape(B, Sq, H * Dh) @ wo

    def _B_ref(x, k_cache, v_cache, wq, wo):
        B, Sq, D = x.shape
        H, Dh = 32, 128
        q = (lambda x, *d: x.transpose(*d))((x @ wq).reshape(B, Sq, H, Dh), 0, 2, 1, 3)
        scores = jnp.einsum("bhqd,bhkd->bhqk", q, k_cache) * (Dh ** -0.5)
        p = _softmax(scores, axis=-1)
        o = jnp.einsum("bhqk,bhkd->bhqd", p, v_cache)
        return (lambda x, *d: x.transpose(*d))(o, 0, 2, 1, 3).reshape(B, Sq, H * Dh) @ wo

    a = _A_ref(A_x, A_k_cache, A_v_cache, A_wq, A_wo)
    b = _B_ref(B_x, B_k_cache, B_v_cache, B_wq, B_wo)
    return jnp.concatenate([a, b], axis=-1)
```

```python
import functools
import numpy as np
import jax
import jax.numpy as jnp
from jax import lax
import jax.experimental.pallas as pl
import jax.experimental.pallas.tpu as pltpu

B, SQ, D, H, SK, DH = 16, 32, 1024, 32, 32, 128
M = B * SQ
BF = jnp.bfloat16
F32 = jnp.float32
NT = (((1,), (1,)), ((), ()))
TN = (((0,), (0,)), ((), ()))
C_EXP2 = float(DH ** -0.5 * np.log2(np.e))


def a_side(a11, a12, a21, a22):
    return [a11 + a22, a21 + a22, a11, a22, a11 + a12, a21 - a11, a12 - a22]


def b_side(i, b11, b12, b21, b22):
    f = lambda b: b().astype(F32)
    if i == 0: return (f(b11) + f(b22)).astype(BF)
    if i == 1: return b11()
    if i == 2: return (f(b12) - f(b22)).astype(BF)
    if i == 3: return (f(b21) - f(b11)).astype(BF)
    if i == 4: return b22()
    if i == 5: return (f(b11) + f(b12)).astype(BF)
    if i == 6: return (f(b21) + f(b22)).astype(BF)


def strassen_tasks(lhs, blocks, emit):
    s = {}
    prod = lambda i: jnp.dot(lhs(i), b_side(i, *blocks), preferred_element_type=F32)

    def t5(): s["m5"] = prod(4)
    def t3():
        s["m3"] = prod(2)
        emit(0, 1, s["m3"] + s["m5"])
    def t4():
        s["m4"] = prod(3)
        s["d1"] = s["m4"] - s["m5"]
    def t2():
        m2 = prod(1)
        emit(1, 0, m2 + s["m4"])
        s["d2"] = s["m3"] - m2
    def t1():
        m1 = prod(0)
        s["d1"] = s["d1"] + m1
        s["d2"] = s["d2"] + m1
    def t7(): emit(0, 0, s["d1"] + prod(6))
    def t6(): emit(1, 1, s["d2"] + prod(5))
    return [t5, t3, t4, t2, t1, t7, t6]


def run(main, extra, where):
    for j in range(-1, len(main)):
        if j >= 0:
            main[j]()
        for e, w in zip(extra, where):
            if w == j:
                e()


def make(R=2, nodma=False, nobc=True, nosc=False, flags=None, NW=None,
         sw=None, pw=None, xw=None, fsw=None, fpw=None):
    G = 2 * R
    NG = H // G
    T = 2 * NG
    NW = NW or (128 if R >= 4 else 256)
    XB_POS = NG // 2 - 1
    NP = 7 * R
    sw = sw or [1 + 3 * i + (i // 2) for i in range(G)]
    pw = pw or [0 + 3 * i + (i // 2) for i in range(G)]
    xw = xw if xw is not None else [2 + 3 * i + (i // 2) for i in range(G)]

    def kernel(ax, ak, av, awq, awo, bx, bk, bv, bwq, bwo, out_hbm,
               xbuf, xa, wqbuf, wobuf, kbuf, vbuf, qbuf, oa, acc, outbuf, sems, osem):
        xs, ks, vs, wqs, wos = (ax, bx), (ak, bk), (av, bv), (awq, bwq), (awo, bwo)

        class Dummy:
            def start(self): pass
            def wait(self): pass
        mk = (lambda *a: Dummy()) if nodma else pltpu.make_async_copy

        def x_copy(br):
            return mk(xs[br], xbuf.at[br], sems.at[4 * T + br])

        def wq_copy(t, src_t=None):
            s = t if src_t is None else src_t
            return mk(wqs[s // NG].at[:, pl.ds((s % NG) * G * DH, G * DH)], wqbuf.at[t], sems.at[4 * t])

        def k_copy(t, src_t=None):
            s = t if src_t is None else src_t
            return mk(ks[s // NG].at[:, pl.ds((s % NG) * G, G)], kbuf.at[t], sems.at[4 * t + 1])

        def v_copy(t, src_t=None):
            s = t if src_t is None else src_t
            return mk(vs[s // NG].at[:, pl.ds((s % NG) * G, G)], vbuf.at[t], sems.at[4 * t + 2])

        def wo_copy(t, src_t=None):
            s = t if src_t is None else src_t
            return mk(wos[s // NG].at[pl.ds((s % NG) * G * DH, G * DH), :], wobuf.at[t], sems.at[4 * t + 3])

        def out_copy(br, c0, w, si):
            return mk(outbuf.at[br, :, pl.ds(c0, w)], out_hbm.at[:, pl.ds(br * D + c0, w)], osem.at[si])

        def wait(fn, t):
            fn(t, 0).wait()

        lane = lax.broadcasted_iota(jnp.int32, (SK, 128), 1)

        def prep_x_tasks(src, dst, kt):
            if isinstance(kt, int):
                c1, c2 = pl.ds(kt * 128, 128), pl.ds(512 + kt * 128, 128)
            else:
                c1, c2 = pl.ds(pl.multiple_of(kt * 128, 128), 128), pl.ds(pl.multiple_of(512 + kt * 128, 128), 128)

            def task(r):
                r1, r2 = pl.ds(r * 64, 64), pl.ds(256 + r * 64, 64)
                ops = a_side(xbuf[src, r1, c1].astype(F32), xbuf[src, r1, c2].astype(F32),
                             xbuf[src, r2, c1].astype(F32), xbuf[src, r2, c2].astype(F32))
                for i in range(7):
                    xa[dst, i, kt, r1, :] = ops[i].astype(BF)
            return [functools.partial(task, r) for r in range(4)]

        def qproj_tasks(t, pairs=None):
            br = t // NG
            tasks = []
            for p in (range(R) if pairs is None else pairs):
                def emit(r, c, val, p=p):
                    qbuf[2 * p + c, pl.ds(256 * r, 256)] = val.astype(BF)
                blk = lambda r, c, p=p: (lambda: wqbuf[t, pl.ds(512 * r, 512), pl.ds((2 * p + c) * DH, DH)])
                lhs = lambda i: jnp.concatenate([xa[br, i, kt] for kt in range(4)], axis=1)
                tasks += strassen_tasks(lhs, (blk(0, 0), blk(0, 1), blk(1, 0), blk(1, 1)), emit)
            return tasks

        def score_tasks(t, ps):
            def task(h):
                for b in range(4):
                    kk = kbuf[t, 4 * b:4 * b + 4, h].reshape(128, DH)
                    qq = qbuf[h, b * 128:(b + 1) * 128, :]
                    st = lax.dot_general(kk, qq, NT, preferred_element_type=F32)
                    c = jnp.where(lane < 64,
                                  jnp.where(lane < 32, st[0:32], st[32:64]),
                                  jnp.where(lane < 96, st[64:96], st[96:128]))
                    m = jnp.max(c, axis=0, keepdims=True)
                    e = jnp.exp2((c - m) * C_EXP2)
                    l = jnp.sum(e, axis=0, keepdims=True)
                    ps[h, b] = e * (1.0 / l)
            return [functools.partial(task, h) for h in range(G)]

        def pv1(t, h, b, ps):
            vv = vbuf[t, 4 * b:4 * b + 4, h].reshape(128, DH)
            pt = jnp.concatenate(
                [jnp.where((lane >= 32 * i) & (lane < 32 * i + 32), ps[h, b], 0.0) for i in range(4)], axis=0).astype(BF)
            return lax.dot_general(pt, vv, TN, preferred_element_type=F32)

        def pv_tasks(t, ps):
            def task(p, b):
                ops = a_side(pv1(t, 2 * p, b, ps), pv1(t, 2 * p + 1, b, ps),
                             pv1(t, 2 * p, b + 2, ps), pv1(t, 2 * p + 1, b + 2, ps))
                for i in range(7):
                    oa[i, p, b * 128:(b + 1) * 128, :] = ops[i].astype(BF)
            return [functools.partial(task, p, b) for p in range(R) for b in range(2)]

        def oproj_tasks(t, final=False):
            br = t // NG
            first = (t % NG) == 0
            tasks = []
            for n in range(512 // NW):
                def emit(r, c, part, n=n):
                    rs, cc = pl.ds(256 * r, 256), pl.ds(512 * c + n * NW, NW)
                    if isinstance(first, bool):
                        new = part if first else acc[rs, cc] + part
                    else:
                        new = jnp.where(first, 0.0, acc[rs, cc]) + part
                    if not final:
                        acc[rs, cc] = new
                    if final or not isinstance(t, int):
                        outbuf[br, rs, cc] = new.astype(BF)
                    if final and r == c:
                        out_copy(1, 512 * c + n * NW, NW, 1 + 2 * n + c).start()
                blk = lambda odd, c, n=n: (lambda: jnp.concatenate(
                    [wobuf[t, pl.ds((2 * p + odd) * DH, DH), pl.ds(512 * c + n * NW, NW)] for p in range(R)], axis=0))
                lhs = lambda i: jnp.concatenate([oa[i, p] for p in range(R)], axis=1)
                tasks += strassen_tasks(lhs, (blk(0, 0), blk(0, 1), blk(1, 0), blk(1, 1)), emit)
            return tasks

        x_copy(0).start()
        wq_copy(0).start()
        k_copy(0).start(); wq_copy(1).start(); v_copy(0).start()
        for t in range(1, T):
            k_copy(t).start(); wo_copy(t - 1).start(); v_copy(t).start()
            if t + 1 < T:
                wq_copy(t + 1).start()
            if t == XB_POS:
                x_copy(1).start()
        wo_copy(T - 1).start()

        x_copy(0).wait()
        for kt in range(4):
            for task in prep_x_tasks(0, 0, kt):
                task()
        wait(wq_copy, 0)
        run(qproj_tasks(0), [], [])

        wait(k_copy, 0); wait(wq_copy, 1); wait(v_copy, 0)
        ps = {}
        for task in score_tasks(0, ps):
            task()
        run(qproj_tasks(1), pv_tasks(0, ps), fpw or [1 + 3 * i + (i // 2) for i in range(G)])

        def body(t, c):
            @pl.when(t == XB_POS + 1)
            def _():
                x_copy(1).wait()

            @pl.when(t == NG + 1)
            def _():
                out_copy(0, 0, D, 0).start()
            wait(k_copy, t); wait(wo_copy, t - 1); wait(v_copy, t); wait(wq_copy, t + 1)
            nx = R // 2
            live = jnp.logical_and(t > XB_POS, t <= XB_POS + 4 // nx)
            xt = []
            for j in range(nx):
                xt += prep_x_tasks(jnp.where(live, 1, 0), jnp.where(live, 1, 2), (t % (4 // nx)) * nx + j)
            ps = {}
            run(oproj_tasks(t - 1), score_tasks(t, ps) + xt, sw + xw)
            run(qproj_tasks(t + 1), pv_tasks(t, ps), pw)
            return c
        lax.fori_loop(1, T - 1, body, 0)

        wait(k_copy, T - 1); wait(wo_copy, T - 2); wait(v_copy, T - 1); wait(wo_copy, T - 1)
        ps = {}
        run(oproj_tasks(T - 2), score_tasks(T - 1, ps), fsw or [-1 + 2 * i for i in range(G)])
        for task in pv_tasks(T - 1, ps):
            task()
        run(oproj_tasks(T - 1, final=True), [], [])
        out_copy(0, 0, D, 0).wait()
        for n in range(512 // NW):
            out_copy(1, n * NW, NW, 1 + 2 * n).wait()
            out_copy(1, 512 + n * NW, NW, 2 + 2 * n).wait()

    def f(A_x, A_k, A_v, A_wq, A_wo, B_x, B_k, B_v, B_wq, B_wo):
        anyspec = pl.BlockSpec(memory_space=pl.ANY)
        out = pl.pallas_call(
            kernel,
            in_specs=[anyspec] * 10,
            out_specs=anyspec,
            out_shape=jax.ShapeDtypeStruct((M, 2 * D), BF),
            scratch_shapes=[
                pltpu.VMEM((2, M, D), BF),
                pltpu.VMEM((3, 7, 4, 256, 128), BF),
                pltpu.VMEM((T, D, G * DH), BF),
                pltpu.VMEM((T, G * DH, D), BF),
                pltpu.VMEM((T, B, G, SK, DH), BF),
                pltpu.VMEM((T, B, G, SK, DH), BF),
                pltpu.VMEM((G, M, DH), BF),
                pltpu.VMEM((7, R, 256, DH), BF),
                pltpu.VMEM((M, D), F32),
                pltpu.VMEM((2, M, D), BF),
                pltpu.SemaphoreType.DMA((4 * T + 2,)),
                pltpu.SemaphoreType.DMA((1 + 2 * (512 // NW),)),
            ],
            compiler_params=pltpu.CompilerParams(vmem_limit_bytes=100 * 1024 * 1024, disable_bounds_checks=nobc,
                                                 disable_semaphore_checks=nosc, flags=flags),
        )(A_x.reshape(M, D), A_k, A_v, A_wq, A_wo, B_x.reshape(M, D), B_k, B_v, B_wq, B_wo)
        return out.reshape(B, SQ, 2 * D)
    return f

_f = make()


@jax.jit
def pallas_concat_heads__mha_block_cached__mha_block_cached__near_ridge_kernel(A_x, A_k_cache, A_v_cache, A_wq, A_wo, B_x, B_k_cache, B_v_cache, B_wq, B_wo):
    return _f(A_x, A_k_cache, A_v_cache, A_wq, A_wo, B_x, B_k_cache, B_v_cache, B_wq, B_wo)
```

```python
import functools

import jax
import jax.experimental.pallas as pl
import jax.experimental.pallas.tpu as pltpu
import jax.numpy as jnp
import numpy as np
from jax import lax

B, SQ, D, H, SK, DH = 16, 32, 1024, 32, 32, 128
M = B * SQ
G = 4
NG = H // G
T = 2 * NG
LOOP_START, LOOP_END = 2, T - 4

BF, F32, U32 = jnp.bfloat16, jnp.float32, jnp.uint32
NT = (((1,), (1,)), ((), ()))
TN = (((0,), (0,)), ((), ()))
SCALE_LOG2E = float(DH ** -0.5 * np.log2(np.e))

A_TERMS = (((0, 0), (1, 1), 1), ((1, 0), (1, 1), 1), ((0, 0),), ((1, 1),),
           ((0, 0), (0, 1), 1), ((1, 0), (0, 0), -1), ((0, 1), (1, 1), -1))
B_TERMS = (((0, 0), (1, 1), 1), ((0, 0),), ((0, 1), (1, 1), -1), ((1, 0), (0, 0), -1),
           ((1, 1),), ((0, 0), (0, 1), 1), ((1, 0), (1, 1), 1))
C_TERMS = {(0, 0): {0: 1, 3: 1, 4: -1, 6: 1}, (0, 1): {2: 1, 4: 1},
           (1, 0): {1: 1, 3: 1}, (1, 1): {0: 1, 1: -1, 2: 1, 5: 1}}
PRODUCT_ORDER = (4, 2, 3, 1, 0, 6, 5)


def _operand(terms, block):
    if len(terms) == 1:
        return block(*terms[0], BF)
    first, second, sign = terms
    x, y = block(*first, F32), block(*second, F32)
    return (x + y if sign > 0 else x - y).astype(BF)


def _strassen_tasks(lhs, rhs, emit, init=None, carry=None, order=PRODUCT_ORDER):
    sums = {}
    missing = {q: len(terms) for q, terms in C_TERMS.items()}

    def task(i):
        m = jnp.dot(lhs(i), rhs(i), preferred_element_type=F32)
        if carry is not None:
            m = carry(i, m)
            if m is None:
                return
        for q, terms in C_TERMS.items():
            if i not in terms:
                continue
            if q not in sums and init is not None:
                sums[q] = (init(*q), 1)
            if q not in sums:
                sums[q] = (m, terms[i])
            else:
                total, sign = sums[q]
                if sign < 0:
                    total = m - total
                else:
                    total = total + m if terms[i] > 0 else total - m
                sums[q] = (total, 1)
            missing[q] -= 1
            if missing[q] == 0:
                emit(*q, sums[q][0])

    return [functools.partial(task, i) for i in order]


def _run(main, extra=(), after=()):
    for j in range(-1, len(main)):
        if j >= 0:
            main[j]()
        for task, position in zip(extra, after):
            if position == j:
                task()


def _aligned(index, n):
    return index if isinstance(index, int) else pl.multiple_of(index, n)


def _kernel(ax, ak, av, awq, awo, bx, bk, bv, bwq, bwo, out_hbm,
            xbuf, wqbuf, wobuf, kbuf, vbuf, qbuf, pbuf, obuf, qpart, acc, outbuf, in_sems, out_sems):
    xs, ks, vs, wqs, wos = (ax, bx), (ak, bk), (av, bv), (awq, bwq), (awo, bwo)

    def x_part(blk, c0=0, nc=D):
        return xs[blk].at[:, pl.ds(c0, nc)], xbuf.at[blk, :, pl.ds(c0, nc)]

    def wq_part(t, r0=0, nr=D, h0=0, nh=G):
        return (wqs[t // NG].at[pl.ds(r0, nr), pl.ds(((t % NG) * G + h0) * DH, nh * DH)],
                wqbuf.at[t, pl.ds(r0, nr), pl.ds(h0 * DH, nh * DH)])

    def wo_part(t, n=1):
        return (wos[t // NG].at[pl.ds((t % NG) * G * DH, n * G * DH), :],
                wobuf.at[pl.ds(t * G * DH, n * G * DH), :])

    def k_part(t, n=1):
        return ks[t // NG].at[:, pl.ds((t % NG) * G, n * G)], kbuf.at[:, pl.ds(t * G, n * G)]

    def v_part(t, n=1):
        return vs[t // NG].at[:, pl.ds((t % NG) * G, n * G)], vbuf.at[:, pl.ds(t * G, n * G)]

    def out_copy(blk, r0, nr, c0, nc):
        return pltpu.make_async_copy(outbuf.at[blk, pl.ds(r0, nr), pl.ds(c0, nc)],
                                     out_hbm.at[pl.ds(r0, nr), pl.ds(blk * D + c0, nc)], out_sems.at[blk])

    groups = []

    def fetch(*parts):
        copies = [pltpu.make_async_copy(src, dst, in_sems.at[len(groups)]) for src, dst in parts]
        groups.append(copies)
        for copy in copies:
            copy.start()
        return copies

    def wait(copies):
        for copy in copies:
            copy.wait()

    def load_packed(ref, *index):
        return pltpu.bitcast(ref.bitcast(U32)[index], BF)

    def qproj_tasks(t, pair_groups, chunks=(0, 1, 2, 3), order=PRODUCT_ORDER):
        blk = t // NG
        tasks = []
        for pairs in pair_groups:
            def x_block(r, c, dtype):
                return jnp.concatenate(
                    [xbuf[blk, pl.ds(256 * r, 256), pl.ds((2 * j + c) * 128, 128)].astype(dtype) for j in chunks],
                    axis=1)

            def w_block(r, c, dtype, pairs=pairs):
                return jnp.concatenate(
                    [jnp.concatenate(
                        [wqbuf[t + p // 2, pl.ds((2 * j + r) * 128, 128), pl.ds((2 * (p % 2) + c) * DH, DH)].astype(dtype)
                         for p in pairs], axis=1)
                     for j in chunks], axis=0)

            def carry(i, m, pairs=pairs):
                cols = pl.ds(pairs[0] * DH, len(pairs) * DH)
                if chunks[0] > 0:
                    m = m + qpart[i, :, cols]
                if chunks[-1] == 3:
                    return m
                qpart[i, :, cols] = m

            def emit(r, c, q, pairs=pairs):
                for n, p in enumerate(pairs):
                    qbuf[(t + p // 2) % 2, 2 * (p % 2) + c, pl.ds(256 * r, 256), :] = q[:, n * DH:(n + 1) * DH].astype(BF)

            tasks += _strassen_tasks(lambda i, block=x_block: _operand(A_TERMS[i], block),
                                     lambda i, block=w_block: _operand(B_TERMS[i], block),
                                     emit, carry=carry, order=order)
        return tasks

    lane = lax.broadcasted_iota(jnp.int32, (SK, 128), 1)

    def score_tasks(t, slot=0):
        def task(h):
            for b in range(4):
                k = kbuf[pl.ds(4 * b, 4), t * G + h].reshape(128, DH)
                q = load_packed(qbuf, t % 2, h, pl.ds(64 * b, 64))
                s = lax.dot_general(k, q, NT, preferred_element_type=F32)
                s = jnp.where(lane < 64,
                              jnp.where(lane < 32, s[0:32], s[32:64]),
                              jnp.where(lane < 96, s[64:96], s[96:128]))
                e = jnp.exp2((s - jnp.max(s, axis=0, keepdims=True)) * SCALE_LOG2E)
                pbuf[slot, h, b] = e * pltpu.reciprocal(jnp.sum(e, axis=0, keepdims=True), full_range=False)

        return [functools.partial(task, h) for h in range(G)]

    def pv_tasks(t, slot=0):
        def pv(h, b):
            p = pbuf[slot, h, b]
            p = jnp.concatenate(
                [jnp.where((lane >= 32 * i) & (lane < 32 * i + 32), p, 0.0) for i in range(4)], axis=0)
            v = vbuf[pl.ds(4 * b, 4), t * G + h].reshape(128, DH)
            return lax.dot_general(p.astype(BF), v, TN, preferred_element_type=F32)

        def task(pair, b):
            o = {(r, c): pv(2 * pair + c, b + 2 * r) for r in range(2) for c in range(2)}
            for i in range(7):
                obuf[slot, i, pair, pl.ds(128 * b, 128), :] = _operand(
                    A_TERMS[i], lambda r, c, dtype: o[r, c].astype(dtype))

        return [functools.partial(task, pair, b) for pair in range(2) for b in range(2)]

    b_out_copies = []

    def oproj_tasks(t, slot=0):
        in_loop = not isinstance(t, int)
        first = not in_loop and t % NG == 0
        final = not in_loop and t == T - 1
        tasks = []
        for c0 in (0, 256):
            def w_block(r, c, dtype, c0=c0):
                return jnp.concatenate(
                    [wobuf[pl.ds(_aligned((t * G + 2 * pair + r) * DH, DH), DH), pl.ds(512 * c + c0, 256)].astype(dtype)
                     for pair in range(2)], axis=0)

            def init(r, c, c0=c0):
                prev = acc[pl.ds(256 * r, 256), pl.ds(512 * c + c0, 256)]
                return jnp.where(t % NG == 0, 0.0, prev) if in_loop else prev

            def emit(r, c, total, c0=c0):
                rows, cols = pl.ds(256 * r, 256), pl.ds(512 * c + c0, 256)
                if final:
                    outbuf[1, rows, cols] = total.astype(BF)
                    b_out_copies.append(out_copy(1, 256 * r, 256, 512 * c + c0, 256))
                    b_out_copies[-1].start()
                    return
                acc[rows, cols] = total
                if in_loop:
                    outbuf[jnp.where(t == NG - 1, 0, 1), rows, cols] = total.astype(BF)

            tasks += _strassen_tasks(
                lambda i: jnp.concatenate([load_packed(obuf, slot, i, pair) for pair in range(2)], axis=1),
                lambda i, block=w_block: _operand(B_TERMS[i], block),
                emit, init=None if first else init)
        return tasks

    def qproj_with_pv(t):
        _run(qproj_tasks(t + 2, ((0,), (1,))), pv_tasks(t), (0, 3, 7, 10))

    def oproj_with_scores(t):
        _run(oproj_tasks(t), score_tasks(t + 1), (1, 4, 8, 11))

    chunk0 = (fetch(x_part(0, 0, 256), wq_part(0, 0, 128), wq_part(1, 0, 128)),
              fetch(wq_part(0, 128, 128), wq_part(1, 128, 128)))
    chunk = {j: fetch(x_part(0, 256 * j, 256), wq_part(0, 256 * j, 256), wq_part(1, 256 * j, 256))
             for j in (1, 2, 3)}
    ramp = (fetch(k_part(0), wq_part(2, h0=0, nh=2)),
            fetch(v_part(0), wq_part(2, h0=2, nh=2)),
            fetch(k_part(1), wo_part(0)),
            fetch(v_part(1), wq_part(3)),
            fetch(k_part(2), wo_part(1)))
    first_loop_group = len(groups)
    x_b = pltpu.make_async_copy(*x_part(1), in_sems.at[in_sems.shape[0] - 1])
    for t in range(LOOP_START, LOOP_END):
        if t == NG - 2:
            x_b.start()
        fetch(v_part(t), wq_part(t + 2), k_part(t + 1), wo_part(t))
    rest = fetch(v_part(LOOP_END, T - LOOP_END), k_part(LOOP_END + 1, T - LOOP_END - 1),
                 wo_part(LOOP_END, T - LOOP_END), *[wq_part(t) for t in range(LOOP_END + 2, T)])

    wait(chunk0[0])
    _run(qproj_tasks(0, ((0, 1, 2, 3),), (0,), order=(1, 5, 4, 2, 3, 0, 6)), [lambda: wait(chunk0[1])], [1])
    for j in (1, 2):
        wait(chunk[j])
        _run(qproj_tasks(0, ((0, 1, 2, 3),), (j,)))
    wait(chunk[3])
    _run(qproj_tasks(0, ((0, 1), (2, 3)), (3,)))
    wait(ramp[0])
    _run(qproj_tasks(2, ((0,),)), score_tasks(0), (-1, 0, 1, 2))
    wait(ramp[1])
    _run(qproj_tasks(2, ((1,),)), pv_tasks(0), (0, 2, 3, 5))
    wait(ramp[2])
    oproj_with_scores(0)
    wait(ramp[3])
    qproj_with_pv(1)
    wait(ramp[4])
    oproj_with_scores(1)

    a_out_copy = out_copy(0, 0, M, 0, D)

    def step(t, carry):
        @pl.when(t == NG - 2)
        def _():
            x_b.wait()

        @pl.when(t == NG)
        def _():
            a_out_copy.start()

        sem = in_sems.at[first_loop_group + t - LOOP_START]
        for dst in (vbuf.at[:, pl.ds(t * G, G)], wqbuf.at[t + 2], kbuf.at[:, pl.ds((t + 1) * G, G)],
                    wobuf.at[pl.ds(_aligned(t * G * DH, G * DH), G * DH), :]):
            pltpu.make_async_copy(dst, dst, sem).wait()
        qproj_with_pv(t)
        oproj_with_scores(t)
        return carry

    lax.fori_loop(LOOP_START, LOOP_END, step, 0)

    wait(rest)
    for t in range(LOOP_END, T - 2):
        qproj_with_pv(t)
        oproj_with_scores(t)
    _run(pv_tasks(T - 2), score_tasks(T - 1, slot=1), (-1, 0, 1, 2))
    _run(oproj_tasks(T - 2), pv_tasks(T - 1, slot=1), (2, 5, 8, 11))
    _run(oproj_tasks(T - 1, slot=1))
    wait([a_out_copy] + b_out_copies)


@jax.jit
def pallas_concat_heads__mha_block_cached__mha_block_cached__near_ridge_kernel(
    A_x: jax.Array,
    A_k_cache: jax.Array,
    A_v_cache: jax.Array,
    A_wq: jax.Array,
    A_wo: jax.Array,
    B_x: jax.Array,
    B_k_cache: jax.Array,
    B_v_cache: jax.Array,
    B_wq: jax.Array,
    B_wo: jax.Array,
):
    hbm = pl.BlockSpec(memory_space=pl.ANY)
    out = pl.pallas_call(
        _kernel,
        in_specs=[hbm] * 10,
        out_specs=hbm,
        out_shape=jax.ShapeDtypeStruct((M, 2 * D), BF),
        scratch_shapes=[
            pltpu.VMEM((2, M, D), BF),
            pltpu.VMEM((T, D, G * DH), BF),
            pltpu.VMEM((2 * H * DH, D), BF),
            pltpu.VMEM((B, 2 * H, SK, DH), BF),
            pltpu.VMEM((B, 2 * H, SK, DH), BF),
            pltpu.VMEM((2, G, M, DH), BF),
            pltpu.VMEM((2, G, 4, SK, 128), F32),
            pltpu.VMEM((2, 7, 2, M // 2, DH), BF),
            pltpu.VMEM((7, M // 2, 4 * DH), F32),
            pltpu.VMEM((M, D), F32),
            pltpu.VMEM((2, M, D), BF),
            pltpu.SemaphoreType.DMA((LOOP_END - LOOP_START + 12,)),
            pltpu.SemaphoreType.DMA((2,)),
        ],
        compiler_params=pltpu.CompilerParams(
            vmem_limit_bytes=100 * 1024 * 1024,
            disable_bounds_checks=True,
            disable_semaphore_checks=True,
        ),
    )(A_x.reshape(M, D), A_k_cache, A_v_cache, A_wq, A_wo,
      B_x.reshape(M, D), B_k_cache, B_v_cache, B_wq, B_wo)
    return out.reshape(B, SQ, 2 * D)
```

```python
import functools

import jax
import jax.experimental.pallas as pl
import jax.experimental.pallas.tpu as pltpu
import jax.numpy as jnp
import numpy as np
from jax import lax

B, SQ, D, H, SK, DH = 16, 32, 1024, 32, 32, 128
M = B * SQ
G = 4
NG = H // G
T = 2 * NG
LOOP_START, UNROLL, ITERATIONS = 2, 3, 4

BF, F32 = jnp.bfloat16, jnp.float32
NT = (((1,), (1,)), ((), ()))
TN = (((0,), (0,)), ((), ()))
SCALE_LOG2E = float(DH ** -0.5 * np.log2(np.e))

A_TERMS = (((0, 0), (1, 1), 1), ((1, 0), (1, 1), 1), ((0, 0),), ((1, 1),),
           ((0, 0), (0, 1), 1), ((1, 0), (0, 0), -1), ((0, 1), (1, 1), -1))
B_TERMS = (((0, 0), (1, 1), 1), ((0, 0),), ((0, 1), (1, 1), -1), ((1, 0), (0, 0), -1),
           ((1, 1),), ((0, 0), (0, 1), 1), ((1, 0), (1, 1), 1))
C_TERMS = {(0, 0): {0: 1, 3: 1, 4: -1, 6: 1}, (0, 1): {2: 1, 4: 1},
           (1, 0): {1: 1, 3: 1}, (1, 1): {0: 1, 1: -1, 2: 1, 5: 1}}
PRODUCT_ORDER = (4, 2, 3, 1, 0, 6, 5)


def _combine(terms, block):
    if len(terms) == 1:
        return block(*terms[0])
    first, second, sign = terms
    return block(*first) + block(*second) if sign > 0 else block(*first) - block(*second)


def _operand(terms, block):
    dtype = BF if len(terms) == 1 else F32
    return _combine(terms, lambda r, c: block(r, c, dtype)).astype(BF)


def _strassen_tasks(lhs, rhs, emit, init=None, carry=None, order=PRODUCT_ORDER):
    sums = {}
    missing = {q: len(terms) for q, terms in C_TERMS.items()}

    def task(i):
        m = jnp.dot(lhs(i), rhs(i), preferred_element_type=F32)
        if carry is not None:
            m = carry(i, m)
            if m is None:
                return
        for q, terms in C_TERMS.items():
            if i not in terms:
                continue
            if q not in sums and init is not None:
                sums[q] = (init(*q), 1)
            if q not in sums:
                sums[q] = (m, terms[i])
            else:
                total, sign = sums[q]
                if sign < 0:
                    total = m - total
                else:
                    total = total + m if terms[i] > 0 else total - m
                sums[q] = (total, 1)
            missing[q] -= 1
            if missing[q] == 0:
                emit(*q, sums[q][0])

    return [functools.partial(task, i) for i in order]


def _run(main, extra=(), after=()):
    for j in range(-1, len(main)):
        if j >= 0:
            main[j]()
        for task, position in zip(extra, after):
            if position == j:
                task()


def _aligned(index, n):
    return index if isinstance(index, int) else pl.multiple_of(index, n)


def _kernel(ax, ak, av, awq, awo, bx, bk, bv, bwq, bwo, out_hbm,
            xbuf, wqbuf, wobuf, kbuf, vbuf, qbuf, pbuf, qpart, acc, outbuf, in_sems, out_sems):
    xs, ks, vs, wqs, wos = (ax, bx), (ak, bk), (av, bv), (awq, bwq), (awo, bwo)

    def x_part(blk, c0=0, nc=D):
        return xs[blk].at[:, pl.ds(c0, nc)], xbuf.at[blk, :, pl.ds(c0, nc)]

    def wq_part(t, r0=0, nr=D):
        src = wqs[t // NG].at[pl.ds(r0, nr), pl.ds(t % NG * G * DH, G * DH)] if isinstance(t, int) else None
        return src, wqbuf.at[t, pl.ds(r0, nr), :]

    def wo_part(t, h0=0, nh=G):
        src = wos[t // NG].at[pl.ds((t % NG * G + h0) * DH, nh * DH), :] if isinstance(t, int) else None
        return src, wobuf.at[pl.ds(_aligned((t * G + h0) * DH, DH), nh * DH), :]

    def k_part(t, nh=G):
        src = ks[t // NG].at[:, pl.ds(t % NG * G, nh)] if isinstance(t, int) else None
        return src, kbuf.at[:, pl.ds(t * G, nh)]

    def v_part(t, nh=G):
        src = vs[t // NG].at[:, pl.ds(t % NG * G, nh)] if isinstance(t, int) else None
        return src, vbuf.at[:, pl.ds(t * G, nh)]

    groups = []

    def fetch(*parts):
        copies = [pltpu.make_async_copy(src, dst, in_sems.at[len(groups)]) for src, dst in parts]
        groups.append(copies)
        for copy in copies:
            copy.start()
        return copies

    def wait(copies):
        for copy in copies:
            copy.wait()

    def out_copy(blk, r0, nr, c0, nc):
        return pltpu.make_async_copy(outbuf.at[blk, pl.ds(r0, nr), pl.ds(c0, nc)],
                                     out_hbm.at[pl.ds(r0, nr), pl.ds(blk * D + c0, nc)], out_sems.at[blk])

    def q_slot(t):
        return t + 2 if isinstance(t, int) and t < 2 else t % 2

    def qproj_tasks(t, pair_groups, chunks=(0, 1, 2, 3), order=PRODUCT_ORDER):
        blk = t // NG
        tasks = []
        for pairs in pair_groups:
            def x_block(r, c, dtype):
                return jnp.concatenate(
                    [xbuf[blk, pl.ds(256 * r, 256), pl.ds((2 * j + c) * 128, 128)].astype(dtype) for j in chunks],
                    axis=1)

            def w_block(r, c, dtype, pairs=pairs):
                return jnp.concatenate(
                    [jnp.concatenate(
                        [wqbuf[t + p // 2, pl.ds((2 * j + r) * 128, 128), pl.ds((2 * (p % 2) + c) * DH, DH)].astype(dtype)
                         for p in pairs], axis=1)
                     for j in chunks], axis=0)

            def carry(i, m, pairs=pairs):
                cols = pl.ds(pairs[0] * DH, len(pairs) * DH)
                if chunks[0] > 0:
                    m = m + qpart[i, :, cols]
                if chunks[-1] == 3:
                    return m
                qpart[i, :, cols] = m

            def emit(r, c, q, pairs=pairs):
                for n, p in enumerate(pairs):
                    qbuf[q_slot(t + p // 2), 2 * (p % 2) + c, pl.ds(256 * r, 256), :] = q[:, n * DH:(n + 1) * DH].astype(BF)

            tasks += _strassen_tasks(lambda i, block=x_block: _operand(A_TERMS[i], block),
                                     lambda i, block=w_block: _operand(B_TERMS[i], block),
                                     emit, carry=carry, order=order)
        return tasks

    lane = lax.broadcasted_iota(jnp.int32, (SK, 128), 1)

    def score_tasks(t, slot=0):
        def task(h):
            for b in range(4):
                k = kbuf[pl.ds(4 * b, 4), t * G + h].reshape(128, DH)
                q = qbuf[q_slot(t), h, pl.ds(128 * b, 128), :]
                s = lax.dot_general(k, q, NT, preferred_element_type=F32)
                s = jnp.where(lane < 64,
                              jnp.where(lane < 32, s[0:32], s[32:64]),
                              jnp.where(lane < 96, s[64:96], s[96:128]))
                e = jnp.exp2((s - jnp.max(s, axis=0, keepdims=True)) * SCALE_LOG2E)
                pbuf[slot, h, b] = e * pltpu.reciprocal(jnp.sum(e, axis=0, keepdims=True), full_range=False)

        return [functools.partial(task, h) for h in range(G)]

    def pv_tasks(t, operands, slot=0):
        pieces = {}

        def pv(h, b):
            p = pbuf[slot, h, b]
            p = jnp.concatenate(
                [jnp.where((lane >= 32 * i) & (lane < 32 * i + 32), p, 0.0) for i in range(4)], axis=0)
            v = vbuf[pl.ds(4 * b, 4), t * G + h].reshape(128, DH)
            return lax.dot_general(p.astype(BF), v, TN, preferred_element_type=F32)

        def task(pair, b):
            o = {(r, c): pv(2 * pair + c, b + 2 * r) for r in range(2) for c in range(2)}
            pieces[pair, b] = [_combine(terms, lambda r, c: o[r, c]) for terms in A_TERMS]
            if len(pieces) == 4:
                operands.extend(
                    jnp.concatenate([jnp.concatenate([pieces[p, 0][i], pieces[p, 1][i]], axis=0) for p in range(2)],
                                    axis=1).astype(BF) for i in range(7))

        return [functools.partial(task, pair, b) for pair in range(2) for b in range(2)]

    b_out_copies = []

    def oproj_tasks(t, operands, may_end_a=False):
        in_loop = not isinstance(t, int)
        first = not in_loop and t % NG == 0
        final = not in_loop and t == T - 1
        tasks = []
        for c0 in (0, 256):
            def w_block(r, c, dtype, c0=c0):
                return jnp.concatenate(
                    [wobuf[pl.ds(_aligned((t * G + 2 * pair + r) * DH, DH), DH), pl.ds(512 * c + c0, 256)].astype(dtype)
                     for pair in range(2)], axis=0)

            def init(r, c, c0=c0):
                prev = acc[pl.ds(256 * r, 256), pl.ds(512 * c + c0, 256)]
                return jnp.where(t % NG == 0, 0.0, prev) if in_loop else prev

            def emit(r, c, total, c0=c0):
                rows, cols = pl.ds(256 * r, 256), pl.ds(512 * c + c0, 256)
                if final:
                    outbuf[1, rows, cols] = total.astype(BF)
                    b_out_copies.append(out_copy(1, 256 * r, 256, 512 * c + c0, 256))
                    b_out_copies[-1].start()
                    return
                acc[rows, cols] = total
                if may_end_a:
                    outbuf[jnp.where(t == NG - 1, 0, 1), rows, cols] = total.astype(BF)

            tasks += _strassen_tasks(lambda i: operands[i], lambda i, block=w_block: _operand(B_TERMS[i], block),
                                     emit, init=None if first else init)
        return tasks

    def iteration_parts(t):
        return ((v_part(t), wq_part(t + 2)),
                (wo_part(t), k_part(t + 1), wq_part(t + 3, 0, D // 2)),
                (v_part(t + 1), wq_part(t + 3, D // 2, D // 2), wo_part(t + 1), k_part(t + 2)),
                (v_part(t + 2), wq_part(t + 4), wo_part(t + 2), k_part(t + 3)))

    wq_chunk = lambda t, j: wq_part(t, 256 * j, 256)
    q_ramp = (
        (fetch(x_part(0, 0, 256), wq_chunk(0, 0)), ((0, 1),), 0),
        (fetch(wq_chunk(1, 0)), ((2, 3),), 0),
        (fetch(wq_chunk(2, 0), wq_chunk(3, 0)), ((4, 5, 6, 7),), 0),
        (fetch(x_part(0, 256, 256), wq_chunk(0, 1), wq_chunk(1, 1)), ((0, 1, 2, 3),), 1),
        (fetch(wq_chunk(2, 1), wq_chunk(3, 1)), ((4, 5, 6, 7),), 1),
        (fetch(x_part(0, 512, 512), wq_chunk(0, 2), wq_chunk(1, 2)), ((0, 1, 2, 3),), 2),
        (fetch(wq_chunk(2, 2), wq_chunk(3, 2)), ((4, 5, 6, 7),), 2),
        (fetch(wq_chunk(0, 3), wq_chunk(1, 3)), ((0, 1), (2, 3)), 3),
        (fetch(wq_chunk(2, 3), wq_chunk(3, 3)), ((4, 5), (6, 7)), 3))
    o_ramp = (fetch(k_part(0), v_part(0)),
              fetch(k_part(1), wo_part(0)),
              fetch(v_part(1), wo_part(1, 0, 2)),
              fetch(wo_part(1, 2, 2), k_part(2)))
    first_loop_group = len(groups)
    for parts in iteration_parts(LOOP_START):
        fetch(*parts)

    for copies, pair_groups, j in q_ramp:
        wait(copies)
        _run(qproj_tasks(0, pair_groups, (j,)))
    wait(o_ramp[0])
    _run(score_tasks(0, slot=1))
    wait(o_ramp[1])
    o0, o1 = [], []
    _run(pv_tasks(0, o0, slot=1), score_tasks(1), (-1, -1, 3, 3))
    _run(oproj_tasks(0, o0), [lambda: wait(o_ramp[2])] + pv_tasks(1, o1), (8, 9, 10, 11, 12))
    wait(o_ramp[3])
    _run(oproj_tasks(1, o1), score_tasks(2), (1, 4, 8, 11))

    x_b = pltpu.make_async_copy(*x_part(1), in_sems.at[in_sems.shape[0] - 1])
    x_b.start()
    for i in range(1, ITERATIONS):
        for parts in iteration_parts(LOOP_START + UNROLL * i):
            fetch(*parts)
    last = fetch(v_part(T - 2, 2 * G), k_part(T - 1), wo_part(T - 2, 0, 2 * G))

    a_out_copy = out_copy(0, 0, M, 0, D)

    def iteration(i, carry):
        t0 = LOOP_START + UNROLL * i

        @pl.when(i == 1)
        def _():
            x_b.wait()

        @pl.when(i == 2)
        def _():
            a_out_copy.start()

        def wait_group(g):
            for _, dst in iteration_parts(t0)[g]:
                pltpu.make_async_copy(dst, dst, in_sems.at[first_loop_group + 4 * i + g]).wait()

        for j in range(UNROLL):
            t, o = t0 + j, []
            wait_group(j + 1 if j else 0)
            _run(qproj_tasks(t + 2, ((0,), (1,))),
                 pv_tasks(t, o) + ([] if j else [lambda: wait_group(1)]), (0, 3, 7, 10, 9))
            _run(oproj_tasks(t, o, may_end_a=j == (NG - 1 - LOOP_START) % UNROLL), score_tasks(t + 1), (1, 4, 8, 11))
        return carry

    lax.fori_loop(0, ITERATIONS, iteration, 0)

    wait(last)
    o0, o1 = [], []
    _run(pv_tasks(T - 2, o0), score_tasks(T - 1, slot=1), (-1, 0, 1, 2))
    _run(oproj_tasks(T - 2, o0), pv_tasks(T - 1, o1, slot=1), (2, 5, 8, 11))
    _run(oproj_tasks(T - 1, o1))
    wait([a_out_copy] + b_out_copies)


@jax.jit
def pallas_concat_heads__mha_block_cached__mha_block_cached__near_ridge_kernel(
    A_x: jax.Array,
    A_k_cache: jax.Array,
    A_v_cache: jax.Array,
    A_wq: jax.Array,
    A_wo: jax.Array,
    B_x: jax.Array,
    B_k_cache: jax.Array,
    B_v_cache: jax.Array,
    B_wq: jax.Array,
    B_wo: jax.Array,
):
    hbm = pl.BlockSpec(memory_space=pl.ANY)
    out = pl.pallas_call(
        _kernel,
        in_specs=[hbm] * 10,
        out_specs=hbm,
        out_shape=jax.ShapeDtypeStruct((M, 2 * D), BF),
        scratch_shapes=[
            pltpu.VMEM((2, M, D), BF),
            pltpu.VMEM((T, D, G * DH), BF),
            pltpu.VMEM((2 * H * DH, D), BF),
            pltpu.VMEM((B, 2 * H, SK, DH), BF),
            pltpu.VMEM((B, 2 * H, SK, DH), BF),
            pltpu.VMEM((4, G, M, DH), BF),
            pltpu.VMEM((2, G, 4, SK, 128), F32),
            pltpu.VMEM((7, M // 2, 8 * DH), F32),
            pltpu.VMEM((M, D), F32),
            pltpu.VMEM((2, M, D), BF),
            pltpu.SemaphoreType.DMA((9 + 4 + 4 * ITERATIONS + 2,)),
            pltpu.SemaphoreType.DMA((2,)),
        ],
        compiler_params=pltpu.CompilerParams(
            vmem_limit_bytes=100 * 1024 * 1024,
            disable_bounds_checks=True,
            disable_semaphore_checks=True,
            flags={"XLA_TPU_RESCHEDULE_DMA_DONES": True},
        ),
    )(A_x.reshape(M, D), A_k_cache, A_v_cache, A_wq, A_wo,
      B_x.reshape(M, D), B_k_cache, B_v_cache, B_wq, B_wo)
    return out.reshape(B, SQ, 2 * D)
```

```python
import functools

import jax
import jax.experimental.pallas as pl
import jax.experimental.pallas.tpu as pltpu
import jax.numpy as jnp
import numpy as np
from jax import lax

B, SQ, D, H, SK, DH = 16, 32, 1024, 32, 32, 128
M = B * SQ
G = 4
NG = H // G
T = 2 * NG
LOOP_START, UNROLL, ITERATIONS = 2, 3, 4

BF, F32 = jnp.bfloat16, jnp.float32
NT = (((1,), (1,)), ((), ()))
TN = (((0,), (0,)), ((), ()))
SCALE_LOG2E = float(DH ** -0.5 * np.log2(np.e))

A_TERMS = (((0, 0), (1, 1), 1), ((1, 0), (1, 1), 1), ((0, 0),), ((1, 1),),
           ((0, 0), (0, 1), 1), ((1, 0), (0, 0), -1), ((0, 1), (1, 1), -1))
B_TERMS = (((0, 0), (1, 1), 1), ((0, 0),), ((0, 1), (1, 1), -1), ((1, 0), (0, 0), -1),
           ((1, 1),), ((0, 0), (0, 1), 1), ((1, 0), (1, 1), 1))
C_TERMS = {(0, 0): {0: 1, 3: 1, 4: -1, 6: 1}, (0, 1): {2: 1, 4: 1},
           (1, 0): {1: 1, 3: 1}, (1, 1): {0: 1, 1: -1, 2: 1, 5: 1}}
PRODUCT_ORDER = (4, 2, 3, 1, 0, 6, 5)


def _combine(terms, block):
    if len(terms) == 1:
        return block(*terms[0])
    first, second, sign = terms
    return block(*first) + block(*second) if sign > 0 else block(*first) - block(*second)


def _operand(terms, block):
    dtype = BF if len(terms) == 1 else F32
    return _combine(terms, lambda r, c: block(r, c, dtype)).astype(BF)


def _strassen_tasks(lhs, rhs, emit, init=None, carry=None, order=PRODUCT_ORDER):
    sums = {}
    missing = {q: len(terms) for q, terms in C_TERMS.items()}

    def task(i):
        m = jnp.dot(lhs(i), rhs(i), preferred_element_type=F32)
        if carry is not None:
            m = carry(i, m)
            if m is None:
                return
        for q, terms in C_TERMS.items():
            if i not in terms:
                continue
            if q not in sums and init is not None:
                sums[q] = (init(*q), 1)
            if q not in sums:
                sums[q] = (m, terms[i])
            else:
                total, sign = sums[q]
                if sign < 0:
                    total = m - total
                else:
                    total = total + m if terms[i] > 0 else total - m
                sums[q] = (total, 1)
            missing[q] -= 1
            if missing[q] == 0:
                emit(*q, sums[q][0])

    return [functools.partial(task, i) for i in order]


def _run(main, extra=(), after=()):
    for j in range(-1, len(main)):
        if j >= 0:
            main[j]()
        for task, position in zip(extra, after):
            if position == j:
                task()


def _aligned(index, n):
    return index if isinstance(index, int) else pl.multiple_of(index, n)


def _kernel(ax, ak, av, awq, awo, bx, bk, bv, bwq, bwo, out_hbm,
            xbuf, wqbuf, wobuf, kbuf, vbuf, qbuf, pbuf, qpart, acc, outbuf, in_sems, out_sems):
    xs, ks, vs, wqs, wos = (ax, bx), (ak, bk), (av, bv), (awq, bwq), (awo, bwo)

    def x_part(blk, c0=0, nc=D):
        return xs[blk].at[:, pl.ds(c0, nc)], xbuf.at[blk, :, pl.ds(c0, nc)]

    def wq_part(t, r0=0, nr=D):
        src = wqs[t // NG].at[pl.ds(r0, nr), pl.ds(t % NG * G * DH, G * DH)] if isinstance(t, int) else None
        return src, wqbuf.at[t, pl.ds(r0, nr), :]

    def wo_part(t, h0=0, nh=G):
        src = wos[t // NG].at[pl.ds((t % NG * G + h0) * DH, nh * DH), :] if isinstance(t, int) else None
        return src, wobuf.at[pl.ds(_aligned((t * G + h0) * DH, DH), nh * DH), :]

    def k_part(t, nh=G):
        src = ks[t // NG].at[:, pl.ds(t % NG * G, nh)] if isinstance(t, int) else None
        return src, kbuf.at[:, pl.ds(t * G, nh)]

    def v_part(t, nh=G):
        src = vs[t // NG].at[:, pl.ds(t % NG * G, nh)] if isinstance(t, int) else None
        return src, vbuf.at[:, pl.ds(t * G, nh)]

    groups = []

    def fetch(*parts):
        copies = [pltpu.make_async_copy(src, dst, in_sems.at[len(groups)]) for src, dst in parts]
        groups.append(copies)
        for copy in copies:
            copy.start()
        return copies

    def wait(copies):
        for copy in copies:
            copy.wait()

    def out_copy(blk, r0, nr, c0, nc):
        return pltpu.make_async_copy(outbuf.at[blk, pl.ds(r0, nr), pl.ds(c0, nc)],
                                     out_hbm.at[pl.ds(r0, nr), pl.ds(blk * D + c0, nc)], out_sems.at[blk])

    def q_slot(t):
        return t + 2 if isinstance(t, int) and t < 2 else t % 2

    def qproj_tasks(t, pair_groups, chunks=(0, 1, 2, 3), order=PRODUCT_ORDER):
        blk = t // NG
        tasks = []
        for pairs in pair_groups:
            def x_block(r, c, dtype):
                return jnp.concatenate(
                    [xbuf[blk, pl.ds(256 * r, 256), pl.ds((2 * j + c) * 128, 128)].astype(dtype) for j in chunks],
                    axis=1)

            def w_block(r, c, dtype, pairs=pairs):
                return jnp.concatenate(
                    [jnp.concatenate(
                        [wqbuf[t + p // 2, pl.ds((2 * j + r) * 128, 128), pl.ds((2 * (p % 2) + c) * DH, DH)].astype(dtype)
                         for p in pairs], axis=1)
                     for j in chunks], axis=0)

            def carry(i, m, pairs=pairs):
                cols = pl.ds(pairs[0] * DH, len(pairs) * DH)
                if chunks[0] > 0:
                    m = m + qpart[i, :, cols]
                if chunks[-1] == 3:
                    return m
                qpart[i, :, cols] = m

            def emit(r, c, q, pairs=pairs):
                for n, p in enumerate(pairs):
                    qbuf[q_slot(t + p // 2), 2 * (p % 2) + c, pl.ds(256 * r, 256), :] = q[:, n * DH:(n + 1) * DH].astype(BF)

            tasks += _strassen_tasks(lambda i, block=x_block: _operand(A_TERMS[i], block),
                                     lambda i, block=w_block: _operand(B_TERMS[i], block),
                                     emit, carry=carry, order=order)
        return tasks

    lane = lax.broadcasted_iota(jnp.int32, (SK, 128), 1)

    def score_tasks(t, slot=0):
        def task(h):
            for b in range(4):
                k = kbuf[pl.ds(4 * b, 4), t * G + h].reshape(128, DH)
                q = qbuf[q_slot(t), h, pl.ds(128 * b, 128), :]
                s = lax.dot_general(k, q, NT, preferred_element_type=F32)
                s = jnp.where(lane < 64,
                              jnp.where(lane < 32, s[0:32], s[32:64]),
                              jnp.where(lane < 96, s[64:96], s[96:128]))
                e = jnp.exp2((s - jnp.max(s, axis=0, keepdims=True)) * SCALE_LOG2E)
                pbuf[slot, h, b] = e * pltpu.reciprocal(jnp.sum(e, axis=0, keepdims=True), full_range=False)

        return [functools.partial(task, h) for h in range(G)]

    def pv_tasks(t, operands, slot=0):
        pieces = {}

        def pv(h, b):
            p = pbuf[slot, h, b]
            p = jnp.concatenate(
                [jnp.where((lane >= 32 * i) & (lane < 32 * i + 32), p, 0.0) for i in range(4)], axis=0)
            v = vbuf[pl.ds(4 * b, 4), t * G + h].reshape(128, DH)
            return lax.dot_general(p.astype(BF), v, TN, preferred_element_type=F32)

        def task(pair, b):
            o = {(r, c): pv(2 * pair + c, b + 2 * r) for r in range(2) for c in range(2)}
            pieces[pair, b] = [_combine(terms, lambda r, c: o[r, c]) for terms in A_TERMS]
            if len(pieces) == 4:
                operands.extend(
                    jnp.concatenate([jnp.concatenate([pieces[p, 0][i], pieces[p, 1][i]], axis=0) for p in range(2)],
                                    axis=1).astype(BF) for i in range(7))

        return [functools.partial(task, pair, b) for pair in range(2) for b in range(2)]

    b_out_copies = []

    def oproj_tasks(t, operands, may_end_a=False):
        in_loop = not isinstance(t, int)
        first = not in_loop and t % NG == 0
        final = not in_loop and t == T - 1
        tasks = []
        for c0 in (0, 256):
            def w_block(r, c, dtype, c0=c0):
                return jnp.concatenate(
                    [wobuf[pl.ds(_aligned((t * G + 2 * pair + r) * DH, DH), DH), pl.ds(512 * c + c0, 256)].astype(dtype)
                     for pair in range(2)], axis=0)

            def init(r, c, c0=c0):
                prev = acc[pl.ds(256 * r, 256), pl.ds(512 * c + c0, 256)]
                return jnp.where(t % NG == 0, 0.0, prev) if in_loop else prev

            def emit(r, c, total, c0=c0):
                rows, cols = pl.ds(256 * r, 256), pl.ds(512 * c + c0, 256)
                if final:
                    outbuf[1, rows, cols] = total.astype(BF)
                    b_out_copies.append(out_copy(1, 256 * r, 256, 512 * c + c0, 256))
                    b_out_copies[-1].start()
                    return
                acc[rows, cols] = total
                if may_end_a:
                    outbuf[jnp.where(t == NG - 1, 0, 1), rows, cols] = total.astype(BF)

            tasks += _strassen_tasks(lambda i: operands[i], lambda i, block=w_block: _operand(B_TERMS[i], block),
                                     emit, init=None if first else init)
        return tasks

    def iteration_parts(t):
        return ((v_part(t), wq_part(t + 2)),
                (wo_part(t), k_part(t + 1), wq_part(t + 3, 0, D // 2)),
                (v_part(t + 1), wq_part(t + 3, D // 2, D // 2), wo_part(t + 1), k_part(t + 2)),
                *[(v_part(t + j), wq_part(t + j + 2), wo_part(t + j), k_part(t + j + 1)) for j in range(2, UNROLL)])

    wq_chunk = lambda t, j: wq_part(t, 256 * j, 256)
    q_ramp = (
        (fetch(x_part(0, 0, 256), wq_chunk(0, 0)), ((0, 1),), 0),
        (fetch(wq_chunk(1, 0)), ((2, 3),), 0),
        (fetch(wq_chunk(2, 0), wq_chunk(3, 0)), ((4, 5, 6, 7),), 0),
        (fetch(x_part(0, 256, 256), wq_chunk(0, 1), wq_chunk(1, 1)), ((0, 1, 2, 3),), 1),
        (fetch(wq_chunk(2, 1), wq_chunk(3, 1)), ((4, 5, 6, 7),), 1),
        (fetch(x_part(0, 512, 512), wq_chunk(0, 2), wq_chunk(1, 2)), ((0, 1, 2, 3),), 2),
        (fetch(wq_chunk(2, 2), wq_chunk(3, 2)), ((4, 5, 6, 7),), 2),
        (fetch(wq_chunk(0, 3), wq_chunk(1, 3)), ((0, 1), (2, 3)), 3),
        (fetch(wq_chunk(2, 3), wq_chunk(3, 3)), ((4, 5), (6, 7)), 3))
    o_ramp = (fetch(k_part(0), v_part(0)),
              fetch(k_part(1), wo_part(0)),
              fetch(v_part(1), wo_part(1, 0, 2)),
              fetch(wo_part(1, 2, 2), k_part(2)))
    first_loop_group = len(groups)
    for parts in iteration_parts(LOOP_START):
        fetch(*parts)

    for copies, pair_groups, j in q_ramp:
        wait(copies)
        _run(qproj_tasks(0, pair_groups, (j,)))
    wait(o_ramp[0])
    _run(score_tasks(0, slot=1))
    wait(o_ramp[1])
    o0, o1 = [], []
    _run(pv_tasks(0, o0, slot=1), score_tasks(1), (-1, -1, 3, 3))
    _run(oproj_tasks(0, o0), [lambda: wait(o_ramp[2])] + pv_tasks(1, o1), (8, 9, 10, 11, 12))
    wait(o_ramp[3])
    _run(oproj_tasks(1, o1), score_tasks(2), (1, 4, 8, 11))

    x_b = pltpu.make_async_copy(*x_part(1), in_sems.at[in_sems.shape[0] - 1])
    x_b.start()
    for i in range(1, ITERATIONS):
        for parts in iteration_parts(LOOP_START + UNROLL * i):
            fetch(*parts)
    last = fetch(v_part(T - 2, 2 * G), k_part(T - 1), wo_part(T - 2, 0, 2 * G))

    a_out_copy = out_copy(0, 0, M, 0, D)

    def iteration(i, carry):
        t0 = LOOP_START + UNROLL * i

        @pl.when(i == 1)
        def _():
            x_b.wait()

        @pl.when(i == 2)
        def _():
            a_out_copy.start()

        def wait_group(g):
            for _, dst in iteration_parts(t0)[g]:
                pltpu.make_async_copy(dst, dst, in_sems.at[first_loop_group + (UNROLL + 1) * i + g]).wait()

        for j in range(UNROLL):
            t, o = t0 + j, []
            wait_group(j + 1 if j else 0)
            _run(qproj_tasks(t + 2, ((0,), (1,))),
                 pv_tasks(t, o) + ([] if j else [lambda: wait_group(1)]), (0, 3, 7, 10, 9))
            _run(oproj_tasks(t, o, may_end_a=j == (NG - 1 - LOOP_START) % UNROLL), score_tasks(t + 1), (1, 4, 8, 11))

        @pl.when(i == ITERATIONS - 1)
        def _():
            wait(last)
            o0, o1 = [], []
            _run(pv_tasks(T - 2, o0), score_tasks(T - 1, slot=1), (-1, 0, 1, 2))
            _run(oproj_tasks(T - 2, o0), pv_tasks(T - 1, o1, slot=1), (2, 5, 8, 11))
            _run(oproj_tasks(T - 1, o1))
            wait([a_out_copy] + b_out_copies)

        return carry

    lax.fori_loop(0, ITERATIONS, iteration, 0)


@jax.jit
def pallas_concat_heads__mha_block_cached__mha_block_cached__near_ridge_kernel(
    A_x: jax.Array,
    A_k_cache: jax.Array,
    A_v_cache: jax.Array,
    A_wq: jax.Array,
    A_wo: jax.Array,
    B_x: jax.Array,
    B_k_cache: jax.Array,
    B_v_cache: jax.Array,
    B_wq: jax.Array,
    B_wo: jax.Array,
):
    hbm = pl.BlockSpec(memory_space=pl.ANY)
    out = pl.pallas_call(
        _kernel,
        in_specs=[hbm] * 10,
        out_specs=hbm,
        out_shape=jax.ShapeDtypeStruct((M, 2 * D), BF),
        scratch_shapes=[
            pltpu.VMEM((2, M, D), BF),
            pltpu.VMEM((T, D, G * DH), BF),
            pltpu.VMEM((2 * H * DH, D), BF),
            pltpu.VMEM((B, 2 * H, SK, DH), BF),
            pltpu.VMEM((B, 2 * H, SK, DH), BF),
            pltpu.VMEM((4, G, M, DH), BF),
            pltpu.VMEM((2, G, 4, SK, 128), F32),
            pltpu.VMEM((7, M // 2, 8 * DH), F32),
            pltpu.VMEM((M, D), F32),
            pltpu.VMEM((2, M, D), BF),
            pltpu.SemaphoreType.DMA((9 + 4 + (UNROLL + 1) * ITERATIONS + 2,)),
            pltpu.SemaphoreType.DMA((2,)),
        ],
        compiler_params=pltpu.CompilerParams(
            vmem_limit_bytes=100 * 1024 * 1024,
            disable_bounds_checks=True,
            disable_semaphore_checks=True,
            flags={"XLA_TPU_RESCHEDULE_DMA_DONES": True},
        ),
    )(A_x.reshape(M, D), A_k_cache, A_v_cache, A_wq, A_wo,
      B_x.reshape(M, D), B_k_cache, B_v_cache, B_wq, B_wo)
    return out.reshape(B, SQ, 2 * D)
```

```python
import functools

import jax
import jax.experimental.pallas as pl
import jax.experimental.pallas.tpu as pltpu
import jax.numpy as jnp
import numpy as np
from jax import lax

B, SQ, D, H, SK, DH = 16, 32, 1024, 32, 32, 128
M = B * SQ
G = 4
NG = H // G
T = 2 * NG
LOOP_START, UNROLL, ITERATIONS = 2, 3, 4

BF, F32 = jnp.bfloat16, jnp.float32
NT = (((1,), (1,)), ((), ()))
TN = (((0,), (0,)), ((), ()))
SCALE_LOG2E = float(DH ** -0.5 * np.log2(np.e))

A_TERMS = (((0, 0), (1, 1), 1), ((1, 0), (1, 1), 1), ((0, 0),), ((1, 1),),
           ((0, 0), (0, 1), 1), ((1, 0), (0, 0), -1), ((0, 1), (1, 1), -1))
B_TERMS = (((0, 0), (1, 1), 1), ((0, 0),), ((0, 1), (1, 1), -1), ((1, 0), (0, 0), -1),
           ((1, 1),), ((0, 0), (0, 1), 1), ((1, 0), (1, 1), 1))
C_TERMS = {(0, 0): {0: 1, 3: 1, 4: -1, 6: 1}, (0, 1): {2: 1, 4: 1},
           (1, 0): {1: 1, 3: 1}, (1, 1): {0: 1, 1: -1, 2: 1, 5: 1}}
PRODUCT_ORDER = (4, 2, 3, 1, 0, 6, 5)


def _combine(terms, block):
    if len(terms) == 1:
        return block(*terms[0])
    first, second, sign = terms
    return block(*first) + block(*second) if sign > 0 else block(*first) - block(*second)


def _operand(terms, block):
    dtype = BF if len(terms) == 1 else F32
    return _combine(terms, lambda r, c: block(r, c, dtype)).astype(BF)


def _strassen_tasks(lhs, rhs, emit, init=None, carry=None):
    sums = {}
    missing = {q: len(terms) for q, terms in C_TERMS.items()}

    def task(i):
        m = jnp.dot(lhs(i), rhs(i), preferred_element_type=F32)
        if carry is not None:
            m = carry(i, m)
            if m is None:
                return
        for q, terms in C_TERMS.items():
            if i not in terms:
                continue
            if q not in sums and init is not None:
                sums[q] = (init(*q), 1)
            if q not in sums:
                sums[q] = (m, terms[i])
            else:
                total, sign = sums[q]
                if sign < 0:
                    total = m - total
                else:
                    total = total + m if terms[i] > 0 else total - m
                sums[q] = (total, 1)
            missing[q] -= 1
            if missing[q] == 0:
                emit(*q, sums[q][0])

    return [functools.partial(task, i) for i in PRODUCT_ORDER]


def _run(main, extra=(), after=()):
    for j in range(-1, len(main)):
        if j >= 0:
            main[j]()
        for task, position in zip(extra, after):
            if position == j:
                task()


def _aligned(index, n):
    return index if isinstance(index, int) else pl.multiple_of(index, n)


def _kernel(ax, ak, av, awq, awo, bx, bk, bv, bwq, bwo, out_hbm,
            xbuf, wqbuf, wobuf, kbuf, vbuf, qbuf, pbuf, qpart, acc, outbuf, in_sems, out_sems):
    xs, ks, vs, wqs, wos = (ax, bx), (ak, bk), (av, bv), (awq, bwq), (awo, bwo)

    def x_part(blk, c0=0, nc=D, r0=0, nr=M):
        return xs[blk].at[pl.ds(r0, nr), pl.ds(c0, nc)], xbuf.at[blk, pl.ds(r0, nr), pl.ds(c0, nc)]

    def wq_part(t, r0=0, nr=D):
        src = wqs[t // NG].at[pl.ds(r0, nr), pl.ds(t % NG * G * DH, G * DH)] if isinstance(t, int) else None
        return src, wqbuf.at[t, pl.ds(r0, nr), :]

    def wo_part(t, h0=0, nh=G):
        src = wos[t // NG].at[pl.ds((t % NG * G + h0) * DH, nh * DH), :] if isinstance(t, int) else None
        return src, wobuf.at[pl.ds(_aligned((t * G + h0) * DH, DH), nh * DH), :]

    def k_part(t, nh=G):
        src = ks[t // NG].at[:, pl.ds(t % NG * G, nh)] if isinstance(t, int) else None
        return src, kbuf.at[:, pl.ds(t * G, nh)]

    def v_part(t, nh=G):
        src = vs[t // NG].at[:, pl.ds(t % NG * G, nh)] if isinstance(t, int) else None
        return src, vbuf.at[:, pl.ds(t * G, nh)]

    groups = []

    def fetch(*parts):
        copies = [pltpu.make_async_copy(src, dst, in_sems.at[len(groups)]) for src, dst in parts]
        groups.append(copies)
        for copy in copies:
            copy.start()
        return copies

    def wait(copies):
        for copy in copies:
            copy.wait()

    def out_copy(blk, r0, nr, c0, nc):
        return pltpu.make_async_copy(outbuf.at[blk, pl.ds(r0, nr), pl.ds(c0, nc)],
                                     out_hbm.at[pl.ds(r0, nr), pl.ds(blk * D + c0, nc)], out_sems.at[blk])

    def q_slot(t):
        return t + 2 if isinstance(t, int) and t < 2 else t % 2

    def qproj_tasks(t, pair_groups, chunks=(0, 1, 2, 3), r0=0, nr=256):
        blk = t // NG
        tasks = []
        for pairs in pair_groups:
            def x_block(r, c, dtype):
                return jnp.concatenate(
                    [xbuf[blk, pl.ds(256 * r + r0, nr), pl.ds((2 * j + c) * 128, 128)].astype(dtype) for j in chunks],
                    axis=1)

            def w_block(r, c, dtype, pairs=pairs):
                return jnp.concatenate(
                    [jnp.concatenate(
                        [wqbuf[t + p // 2, pl.ds((2 * j + r) * 128, 128), pl.ds((2 * (p % 2) + c) * DH, DH)].astype(dtype)
                         for p in pairs], axis=1)
                     for j in chunks], axis=0)

            def carry(i, m, pairs=pairs):
                cols = pl.ds(pairs[0] * DH, len(pairs) * DH)
                if chunks[0] > 0:
                    m = m + qpart[i, pl.ds(r0, nr), cols]
                if chunks[-1] == 3:
                    return m
                qpart[i, pl.ds(r0, nr), cols] = m

            def emit(r, c, q, pairs=pairs):
                for n, p in enumerate(pairs):
                    qbuf[q_slot(t + p // 2), 2 * (p % 2) + c, pl.ds(256 * r, 256), :] = q[:, n * DH:(n + 1) * DH].astype(BF)

            tasks += _strassen_tasks(lambda i, block=x_block: _operand(A_TERMS[i], block),
                                     lambda i, block=w_block: _operand(B_TERMS[i], block),
                                     emit, carry=carry)
        return tasks

    lane = lax.broadcasted_iota(jnp.int32, (SK, 128), 1)

    def score_tasks(t, slot=0):
        def task(h):
            for b in range(4):
                k = kbuf[pl.ds(4 * b, 4), t * G + h].reshape(128, DH)
                q = qbuf[q_slot(t), h, pl.ds(128 * b, 128), :]
                s = lax.dot_general(k, q, NT, preferred_element_type=F32)
                s = jnp.where(lane < 64,
                              jnp.where(lane < 32, s[0:32], s[32:64]),
                              jnp.where(lane < 96, s[64:96], s[96:128]))
                e = jnp.exp2((s - jnp.max(s, axis=0, keepdims=True)) * SCALE_LOG2E)
                pbuf[slot, h, b] = e * pltpu.reciprocal(jnp.sum(e, axis=0, keepdims=True), full_range=False)

        return [functools.partial(task, h) for h in range(G)]

    def pv_tasks(t, operands, slot=0):
        pieces = {}

        def pv(h, b):
            p = pbuf[slot, h, b]
            p = jnp.concatenate(
                [jnp.where((lane >= 32 * i) & (lane < 32 * i + 32), p, 0.0) for i in range(4)], axis=0)
            v = vbuf[pl.ds(4 * b, 4), t * G + h].reshape(128, DH)
            return lax.dot_general(p.astype(BF), v, TN, preferred_element_type=F32)

        def task(pair, b):
            o = {(r, c): pv(2 * pair + c, b + 2 * r) for r in range(2) for c in range(2)}
            pieces[pair, b] = [_combine(terms, lambda r, c: o[r, c]) for terms in A_TERMS]
            if len(pieces) == 4:
                operands.extend(
                    jnp.concatenate([jnp.concatenate([pieces[p, 0][i], pieces[p, 1][i]], axis=0) for p in range(2)],
                                    axis=1).astype(BF) for i in range(7))

        return [functools.partial(task, pair, b) for pair in range(2) for b in range(2)]

    b_out_copies = []

    def oproj_tasks(t, operands, may_end_a=False):
        in_loop = not isinstance(t, int)
        first = not in_loop and t % NG == 0
        final = not in_loop and t == T - 1
        tasks = []
        for c0 in (0, 256):
            def w_block(r, c, dtype, c0=c0):
                return jnp.concatenate(
                    [wobuf[pl.ds(_aligned((t * G + 2 * pair + r) * DH, DH), DH), pl.ds(512 * c + c0, 256)].astype(dtype)
                     for pair in range(2)], axis=0)

            def init(r, c, c0=c0):
                prev = acc[pl.ds(256 * r, 256), pl.ds(512 * c + c0, 256)]
                return jnp.where(t % NG == 0, 0.0, prev) if in_loop else prev

            def emit(r, c, total, c0=c0):
                rows, cols = pl.ds(256 * r, 256), pl.ds(512 * c + c0, 256)
                if final:
                    outbuf[1, rows, cols] = total.astype(BF)
                    b_out_copies.append(out_copy(1, 256 * r, 256, 512 * c + c0, 256))
                    b_out_copies[-1].start()
                    return
                acc[rows, cols] = total
                if may_end_a:
                    outbuf[jnp.where(t == NG - 1, 0, 1), rows, cols] = total.astype(BF)

            tasks += _strassen_tasks(lambda i: operands[i], lambda i, block=w_block: _operand(B_TERMS[i], block),
                                     emit, init=None if first else init)
        return tasks

    def iteration_parts(t):
        return ((v_part(t), wq_part(t + 2)),
                (wo_part(t), k_part(t + 1), wq_part(t + 3, 0, D // 2)),
                (v_part(t + 1), wq_part(t + 3, D // 2, D // 2), wo_part(t + 1), k_part(t + 2)),
                *[(v_part(t + j), wq_part(t + j + 2), wo_part(t + j), k_part(t + j + 1)) for j in range(2, UNROLL)])

    wq_chunk = lambda t, j: wq_part(t, 256 * j, 256)
    q_first = (fetch(x_part(0, 0, 256, 0, 128), x_part(0, 0, 256, 256, 128), wq_chunk(0, 0)),
               fetch(x_part(0, 0, 256, 128, 128), x_part(0, 0, 256, 384, 128)))
    q_ramp = (
        (fetch(wq_chunk(1, 0)), ((2, 3),), 0),
        (fetch(wq_chunk(2, 0)), ((4, 5),), 0),
        (fetch(wq_chunk(3, 0)), ((6, 7),), 0),
        (fetch(x_part(0, 256, 256), wq_chunk(0, 1)), ((0, 1),), 1),
        (fetch(wq_chunk(1, 1)), ((2, 3),), 1),
        (fetch(wq_chunk(2, 1), wq_chunk(3, 1)), ((4, 5, 6, 7),), 1),
        (fetch(x_part(0, 512, 512), wq_chunk(0, 2), wq_chunk(1, 2)), ((0, 1, 2, 3),), 2),
        (fetch(wq_chunk(2, 2), wq_chunk(3, 2)), ((4, 5, 6, 7),), 2),
        (fetch(wq_chunk(0, 3), wq_chunk(1, 3)), ((0, 1), (2, 3)), 3),
        (fetch(wq_chunk(2, 3), wq_chunk(3, 3)), ((4, 5), (6, 7)), 3))
    o_ramp = (fetch(k_part(0), v_part(0)),
              fetch(k_part(1), wo_part(0)),
              fetch(v_part(1), wo_part(1, 0, 2)),
              fetch(wo_part(1, 2, 2), k_part(2)))
    first_loop_group = len(groups)
    for parts in iteration_parts(LOOP_START):
        fetch(*parts)

    for n, copies in enumerate(q_first):
        wait(copies)
        _run(qproj_tasks(0, ((0, 1),), (0,), 128 * n, 128))
    for copies, pair_groups, j in q_ramp:
        wait(copies)
        _run(qproj_tasks(0, pair_groups, (j,)))
    wait(o_ramp[0])
    _run(score_tasks(0, slot=1))
    wait(o_ramp[1])
    o0, o1 = [], []
    _run(pv_tasks(0, o0, slot=1), score_tasks(1), (-1, -1, 3, 3))
    _run(oproj_tasks(0, o0), [lambda: wait(o_ramp[2])] + pv_tasks(1, o1), (8, 9, 10, 11, 12))
    wait(o_ramp[3])
    _run(oproj_tasks(1, o1), score_tasks(2), (1, 4, 8, 11))

    x_b = pltpu.make_async_copy(*x_part(1), in_sems.at[in_sems.shape[0] - 1])
    x_b.start()
    for i in range(1, ITERATIONS):
        for parts in iteration_parts(LOOP_START + UNROLL * i):
            fetch(*parts)
    last = fetch(v_part(T - 2, 2 * G), k_part(T - 1), wo_part(T - 2, 0, 2 * G))

    a_out_copy = out_copy(0, 0, M, 0, D)

    def iteration(i, carry):
        t0 = LOOP_START + UNROLL * i

        @pl.when(i == 1)
        def _():
            x_b.wait()

        @pl.when(i == 2)
        def _():
            a_out_copy.start()

        def wait_group(g):
            for _, dst in iteration_parts(t0)[g]:
                pltpu.make_async_copy(dst, dst, in_sems.at[first_loop_group + (UNROLL + 1) * i + g]).wait()

        for j in range(UNROLL):
            t, o = t0 + j, []
            wait_group(j + 1 if j else 0)
            _run(qproj_tasks(t + 2, ((0,), (1,))),
                 pv_tasks(t, o) + ([] if j else [lambda: wait_group(1)]), (0, 3, 7, 10, 9))
            _run(oproj_tasks(t, o, may_end_a=j == (NG - 1 - LOOP_START) % UNROLL), score_tasks(t + 1), (1, 4, 8, 11))

        @pl.when(i == ITERATIONS - 1)
        def _():
            wait(last)
            o0, o1 = [], []
            _run(pv_tasks(T - 2, o0), score_tasks(T - 1, slot=1), (-1, 0, 1, 2))
            _run(oproj_tasks(T - 2, o0), pv_tasks(T - 1, o1, slot=1), (2, 5, 8, 11))
            _run(oproj_tasks(T - 1, o1))
            wait([a_out_copy] + b_out_copies)

        return carry

    lax.fori_loop(0, ITERATIONS, iteration, 0)


@jax.jit
def pallas_concat_heads__mha_block_cached__mha_block_cached__near_ridge_kernel(
    A_x: jax.Array,
    A_k_cache: jax.Array,
    A_v_cache: jax.Array,
    A_wq: jax.Array,
    A_wo: jax.Array,
    B_x: jax.Array,
    B_k_cache: jax.Array,
    B_v_cache: jax.Array,
    B_wq: jax.Array,
    B_wo: jax.Array,
):
    hbm = pl.BlockSpec(memory_space=pl.ANY)
    out = pl.pallas_call(
        _kernel,
        in_specs=[hbm] * 10,
        out_specs=hbm,
        out_shape=jax.ShapeDtypeStruct((M, 2 * D), BF),
        scratch_shapes=[
            pltpu.VMEM((2, M, D), BF),
            pltpu.VMEM((T, D, G * DH), BF),
            pltpu.VMEM((2 * H * DH, D), BF),
            pltpu.VMEM((B, 2 * H, SK, DH), BF),
            pltpu.VMEM((B, 2 * H, SK, DH), BF),
            pltpu.VMEM((4, G, M, DH), BF),
            pltpu.VMEM((2, G, 4, SK, 128), F32),
            pltpu.VMEM((7, M // 2, 8 * DH), F32),
            pltpu.VMEM((M, D), F32),
            pltpu.VMEM((2, M, D), BF),
            pltpu.SemaphoreType.DMA((12 + 4 + (UNROLL + 1) * ITERATIONS + 2,)),
            pltpu.SemaphoreType.DMA((2,)),
        ],
        compiler_params=pltpu.CompilerParams(
            vmem_limit_bytes=100 * 1024 * 1024,
            disable_bounds_checks=True,
            disable_semaphore_checks=True,
            flags={"XLA_TPU_RESCHEDULE_DMA_DONES": True},
        ),
    )(A_x.reshape(M, D), A_k_cache, A_v_cache, A_wq, A_wo,
      B_x.reshape(M, D), B_k_cache, B_v_cache, B_wq, B_wo)
    return out.reshape(B, SQ, 2 * D)
```
